```python
import jax
import jax.numpy as jnp

def _softmax(x, axis=-1):
    return jax.nn.softmax(x, axis=axis)
def _gelu(x):
    return jax.nn.gelu(x, approximate=True)
def _silu(x):
    return jax.nn.silu(x)
def _sigmoid(x):
    return jax.nn.sigmoid(x)
def _layernorm(x, axis=-1, eps=1e-5):
    m = jnp.mean(x, axis=axis, keepdims=True)
    v = jnp.var(x, axis=axis, keepdims=True)
    return (x - m) / jnp.sqrt(v + eps)
def _scatter_add(tgt, idx, src, axis=0):
    return tgt.at[idx].add(src)
def _segment_sum(src, seg, n):
    return jax.ops.segment_sum(src, seg, n)
class _Rng:
    def __init__(self, key):
        self._k = key
    def _next(self):
        self._k, sub = jax.random.split(self._k)
        return sub
    def normal(self, shape):
        return jax.random.normal(self._next(), shape, dtype=jnp.bfloat16)
    def randint(self, lo, hi, shape):
        return jax.random.randint(self._next(), shape, lo, hi, dtype=jnp.int32)
    def uniform(self, shape, lo=0.0, hi=1.0):
        return jax.random.uniform(self._next(), shape, jnp.bfloat16, lo, hi)
    def permutation(self, n):
        return jax.random.permutation(self._next(), n)


kernel_name = 'gated_mix__sliding_block_cached__glu_gated_swiglu__decode'

def setup_inputs():
    _rng = _Rng(jax.random.key(int.from_bytes(__import__("os").urandom(4), "little")))
    _w = (lambda a: (lambda t: t.astype(jnp.bfloat16) if jnp.issubdtype(t.dtype, jnp.floating) else t)(jnp.asarray(a)))
    def _A_setup():
        B, Sq, D = 1, 1, 640
        Hq, Hkv, Sk, Dh = 32, 32, 32768, 192
        assert Hq % Hkv == 0, (Hq, Hkv)
        return {
            "x": _w((lambda *s: _rng.normal(s) * 0.05)(B, Sq, D)),
            "k_cache": _w((lambda *s: _rng.normal(s) * 0.05)(B, Hkv, Sk, Dh)),
            "v_cache": _w((lambda *s: _rng.normal(s) * 0.05)(B, Hkv, Sk, Dh)),
            "wq": _w((lambda *s: _rng.normal(s) * 0.05)(D, Hq * Dh) * (D ** -0.5)),
            "wo": _w((lambda *s: _rng.normal(s) * 0.05)(Hq * Dh, D) * ((Hq * Dh) ** -0.5)),
        }
    _A_in = _A_setup()

    def _B_setup():
        B, S, D, F = 1, 1, 640, 1536
        return {
            "x": _w((lambda *s: _rng.normal(s) * 0.05)(B, S, D)),
            "w1": _w((lambda *s: _rng.normal(s) * 0.05)(D, F) * (2.0 / D) ** 0.5),
            "w3": _w((lambda *s: _rng.normal(s) * 0.05)(D, F) * (2.0 / D) ** 0.5),
            "w2": _w((lambda *s: _rng.normal(s) * 0.05)(F, D) * (2.0 / F) ** 0.5),
        }
    _B_in = _B_setup()

    return {
        "A_x": _A_in["x"],
        "A_k_cache": _A_in["k_cache"],
        "A_v_cache": _A_in["v_cache"],
        "A_wq": _A_in["wq"],
        "A_wo": _A_in["wo"],
        "B_x": _B_in["x"],
        "B_w1": _B_in["w1"],
        "B_w3": _B_in["w3"],
        "B_w2": _B_in["w2"],
        "gate_w": _w((lambda *s: _rng.normal(s) * 0.05)(640)),
    }

def reference(A_x, A_k_cache, A_v_cache, A_wq, A_wo, B_x, B_w1, B_w3, B_w2, gate_w):
    def _A_ref(x, k_cache, v_cache, wq, wo):
        B, Sq, D = x.shape
        Hq, Dh = 32, 192
        Hkv, Sk = k_cache.shape[1], k_cache.shape[2]
        W = min(4096, max(256, Sk // 4))
        rep = Hq // Hkv
        q = (lambda x, *d: x.transpose(*d))((x @ wq).reshape(B, Sq, Hq, Dh), 0, 2, 1, 3)
        k = jnp.repeat(k_cache[:, :, Sk - W:, :], rep, axis=1)
        v = jnp.repeat(v_cache[:, :, Sk - W:, :], rep, axis=1)
        scores = jnp.einsum("bhqd,bhkd->bhqk", q, k) * (Dh ** -0.5)
        p = _softmax(scores, axis=-1)
        o = jnp.einsum("bhqk,bhkd->bhqd", p, v)
        return (lambda x, *d: x.transpose(*d))(o, 0, 2, 1, 3).reshape(B, Sq, Hq * Dh) @ wo

    def _B_ref(x, w1, w3, w2):
        gate = jnp.einsum("bsd,df->bsf", x, w1)
        up = jnp.einsum("bsd,df->bsf", x, w3)
        h = _silu(gate) * up
        out = jnp.einsum("bsf,fd->bsd", h, w2)
        return out

    x = A_x
    g = _sigmoid((x * gate_w).sum(-1, keepdims=True))
    a = _A_ref(x, A_k_cache, A_v_cache, A_wq, A_wo)
    b = _B_ref(x, B_w1, B_w3, B_w2)
    return g * a + (1 - g) * b
```

```python
import jax
import jax.numpy as jnp
from jax import lax
import jax.experimental.pallas as pl
import jax.experimental.pallas.tpu as pltpu

_F32 = jnp.float32
_BF16 = jnp.bfloat16

_PRIO = (0, 1, 1)
_AHEAD = 36
_LANDED = 64
_LOOK = 10
_SLOTS = 16
_CW = 1024
_PT = _CW // 128
_STRIDE = 256
_TAIL = (8, 4, 3)


def _tiles(a):
    R, C = a.shape
    return a.reshape(R // 8, 8, C // 128, 128).transpose(0, 2, 1, 3).reshape(-1, 8, 128)


def _passes(*ntiles):
    return [[(a, t) for a, n in enumerate(ntiles) for t in range(c, n, _STRIDE)]
            for c in range(0, _STRIDE, _PT)]


@jax.jit
def pallas_gated_mix__sliding_block_cached__glu_gated_swiglu__decode_kernel(
    A_x: jax.Array,
    A_k_cache: jax.Array,
    A_v_cache: jax.Array,
    A_wq: jax.Array,
    A_wo: jax.Array,
    B_x: jax.Array,
    B_w1: jax.Array,
    B_w3: jax.Array,
    B_w2: jax.Array,
    gate_w: jax.Array,
):
    del B_x
    B, Sq, D = A_x.shape
    _, H, SK, DH = A_k_cache.shape
    F = B_w1.shape[1]
    W = min(4096, max(256, SK // 4))
    scale = DH ** -0.5
    GS = DH // 8
    NU = W // _CW * H
    ND, NF = D // 128, F // 128
    NQT, NFT = D * H * DH // 1024, D * F // 1024
    PER = len(_PRIO)
    assert B == 1 and Sq == 1 and A_wq.shape[1] == H * DH
    assert H & (H - 1) == 0 and _SLOTS & (_SLOTS - 1) == 0 and NU % _SLOTS == 0
    assert W % _CW == 0 and SK % _CW == 0 and (H * DH) % _CW == 0 and NFT % _PT == 0
    assert _AHEAD % PER == 0 and GS % PER == 0 and _PRIO[0] == 0
    assert _LOOK + pl.cdiv(_AHEAD, GS) < _SLOTS

    kT = jnp.swapaxes(A_k_cache, 2, 3).reshape(H * DH, SK)
    vT = jnp.swapaxes(A_v_cache, 2, 3).reshape(H * DH, SK)

    q_list = sum(_passes(NQT), [])
    f_list = sum(_passes(NFT, NFT, NFT), [])
    o_list = sum(_passes(NQT), [])
    F0 = len(q_list)
    K0 = F0 + len(f_list)
    O0 = K0 + 2 * NU * GS
    NTOT = O0 + len(o_list)
    assert K0 % PER == 0
    last = len(o_list) - sum(_TAIL)
    ends = list(range(NQT // _STRIDE, last, NQT // _STRIDE)) + [last]
    for n in _TAIL:
        ends.append(ends[-1] + n)
    o_groups = list(zip([0] + ends[:-1], ends))
    o_group_of = [g for g, (a, b) in enumerate(o_groups) for _ in range(a, b)]

    def kernel(x_ref, k_ref, v_ref, wq_ref, wo_ref, w1_ref, w3_ref, w2_ref, gw_ref, out_ref,
               kv_b, wq_b, f_b, wo_b, x_b, gw_b, q_f, q_s, s_s, m_s, l_s, o_s, x_s, h_s):

        def body(wsem, kvsem, osem):
            def aligned(i, n):
                return i if isinstance(i, int) else pl.multiple_of(i, n)

            def kv_copy(m, u, r):
                row = aligned((u & (H - 1)) * DH + r * 8, 8)
                col = aligned(SK - W + (u >> (H.bit_length() - 1)) * _CW, _CW)
                slot = u & (_SLOTS - 1)
                return pltpu.make_async_copy((k_ref, v_ref)[m].at[pl.ds(row, 8), pl.ds(col, _CW)],
                                             kv_b.at[slot, pl.ds(r * 8, 8)], kvsem.at[slot])

            def copy(i):
                if i < F0:
                    tr, tc = divmod(q_list[i][1], H * DH // 128)
                    idx = (pl.ds(tr * 8, 8), pl.ds(tc * 128, _CW))
                    return pltpu.make_async_copy(wq_ref.at[idx], wq_b.at[idx], wsem.at[0])
                if i < K0:
                    a, t = f_list[i - F0]
                    return pltpu.make_async_copy((w1_ref, w3_ref, w2_ref)[a].at[pl.ds(t, _PT)],
                                                 f_b.at[a, pl.ds(t, _PT)], wsem.at[1])
                if i < O0:
                    m, j = divmod(i - K0, NU * GS)
                    return kv_copy(m, j // GS, j % GS)
                j = i - O0
                return pltpu.make_async_copy(wo_ref.at[pl.ds(o_list[j][1], _PT)],
                                             wo_b.at[pl.ds(j * _PT, _PT)], osem.at[o_group_of[j]])

            def piece_at(i):
                return (i, 0) if _PRIO[i % PER] == 0 else (i + _AHEAD, 1)

            pos = [0]

            def start_until(n):
                while pos[0] < n:
                    p, prio = piece_at(pos[0])
                    if p < NTOT:
                        copy(p).start(priority=prio)
                    pos[0] += 1

            def wait_filled(buf, sem):
                pltpu.make_async_copy(buf, buf, sem).wait()

            def run_tasks(tasks, n_end, w0, w1):
                n0, nt = pos[0], len(tasks)
                for k, task in enumerate(tasks):
                    task()
                    start_until(n0 + (n_end - n0) * (k + 1) // nt)
                    for i in range(w0 + (w1 - w0) * k // nt, w0 + (w1 - w0) * (k + 1) // nt):
                        copy(i).wait()

            start_until(1)
            for p in range(_AHEAD):
                if _PRIO[p % PER]:
                    copy(p).start(priority=1)
            x_copy = pltpu.make_async_copy(x_ref, x_b, wsem.at[2])
            gw_copy = pltpu.make_async_copy(gw_ref, gw_b, wsem.at[3])
            x_copy.start(priority=1)
            gw_copy.start(priority=1)
            m_s[...] = jnp.full(m_s.shape, -jnp.inf, _F32)
            l_s[...] = jnp.zeros(l_s.shape, _F32)
            o_s[...] = jnp.zeros(o_s.shape, _F32)
            start_until(F0 * 5 // 8)
            x_copy.wait()
            x = x_b[0]
            xb = jnp.broadcast_to(x, (8, D))
            xf = x.astype(_F32)
            for c in range(0, D, 128):
                x_s[c:c + 128, :] = jnp.transpose(jnp.broadcast_to(xf[:, c:c + 128], (128, 128)))
            start_until(F0 * 5 // 6)
            gw_copy.wait()
            gw = gw_b[...].reshape(1, D).astype(_F32)
            gate = jax.nn.sigmoid(jnp.sum(xf * gw, axis=-1, keepdims=True))
            start_until(F0 + _LANDED)
            wait_filled(wq_b, wsem.at[0])

            def q_task(n0):
                def run():
                    q_f[:, n0:n0 + 512] = jnp.dot(xb, wq_b[:, n0:n0 + 512],
                                                  preferred_element_type=_F32).astype(_BF16)
                return run

            def q_split(h0, h1):
                def run():
                    for h in range(h0, h1):
                        q_s[h] = q_f[:, h * DH:(h + 1) * DH]
                return run

            run_tasks([q_task(n0) for n0 in range(0, H * DH, 512)]
                      + [q_split(H * i // 3, H * (i + 1) // 3) for i in range(3)],
                      K0 + _LANDED, F0, K0)

            def up_task(j):
                def run():
                    r = []
                    for a in range(2):
                        acc = [None, None]
                        for tr in range(D // 8):
                            t = f_b[a, tr * NF + j].astype(_F32) * x_s[tr * 8:(tr + 1) * 8, :]
                            acc[tr % 2] = t if acc[tr % 2] is None else acc[tr % 2] + t
                        r.append(jnp.sum(acc[0] + acc[1], axis=0, keepdims=True))
                    hh = (r[0] * jax.nn.sigmoid(r[0]) * r[1]).astype(_BF16).astype(_F32)
                    h_s[j * 128:(j + 1) * 128, :] = jnp.transpose(
                        jnp.broadcast_to(hh * (1.0 - gate), (128, 128)))
                return run

            run_tasks([up_task(j) for j in range(NF)], K0 + _LOOK * GS, K0, K0 + GS)

            def unit(m, u, m_next, finish, starts):
                h = u & (H - 1)
                buf = kv_b.at[u & (_SLOTS - 1)]

                def wait_next(r0, r1):
                    if m_next is not None:
                        for r in range(r0, r1):
                            kv_copy(m_next, (u + 1) & (NU - 1), r).wait()

                if m == 0:
                    mm = m_s[h]
                    cw = _CW // 4
                    for c in range(4):
                        s = jnp.dot(q_s[h], buf[:, c * cw:(c + 1) * cw],
                                    preferred_element_type=_F32) * scale
                        s_s[u, :, c * cw:(c + 1) * cw] = s
                        for k in range(cw // 128):
                            mm = jnp.maximum(mm, s[:, k * 128:(k + 1) * 128])
                        starts(GS * c // 4, GS * (c + 1) // 4)
                    slot = (u + 1) & (_SLOTS - 1)
                    wait_filled(kv_b.at[slot], kvsem.at[slot])
                    m_s[h] = jnp.broadcast_to(jnp.max(mm, axis=-1, keepdims=True), (8, 128))
                    return

                mx = m_s[h]
                e = [jnp.exp(s_s[u, :, k * 128:(k + 1) * 128] - mx) for k in range(_PT)]
                ll = l_s[h]
                for t in e:
                    ll = ll + t
                l_s[h] = ll
                nc = 5 if finish else 6
                for c in range(nc):
                    for r in range(GS * c // nc, GS * (c + 1) // nc):
                        rows = pl.ds(aligned(h * DH + r * 8, 8), 8)
                        vv = buf[r * 8:(r + 1) * 8, :].astype(_F32)
                        acc = [o_s[rows, :], None]
                        for k in range(_PT):
                            t = vv[:, k * 128:(k + 1) * 128] * e[k]
                            acc[k % 2] = t if acc[k % 2] is None else acc[k % 2] + t
                        o_s[rows, :] = acc[0] + acc[1]
                    starts(GS * c // 6, GS * (c + 1) // 6)
                    wait_next(GS * c // 6, GS * (c + 1) // 6)
                if finish:
                    rows = pl.ds(aligned(h * DH, 8), DH)
                    den = jnp.sum(ll, axis=-1, keepdims=True)[0:1]
                    o = jnp.sum(o_s[rows, :], axis=-1, keepdims=True) / den
                    o_s[rows, :] = jnp.broadcast_to(o.astype(_BF16).astype(_F32) * gate, (DH, 128))
                    starts(GS * 5 // 6, GS)
                    wait_next(GS * 5 // 6, GS)

            def signature(g):
                srcs = []
                for r in range(GS):
                    p, _ = piece_at(K0 + (g + _LOOK) * GS + r)
                    srcs.append((p - K0) // (NU * GS) if p < O0 else -p)
                m_next = (g + 1) // NU if g + 1 < 2 * NU else None
                return g // NU, (m_next if g >= NU else 0), g >= 2 * NU - H, tuple(srcs)

            g0 = 0
            while g0 < 2 * NU:
                sig = signature(g0)
                g1 = g0 + 1
                while g1 < 2 * NU and signature(g1) == sig:
                    g1 += 1
                m, m_next, finish, srcs = sig
                n0 = K0 + (g0 + _LOOK) * GS
                assert pos[0] == n0
                if g1 == g0 + 1:
                    unit(m, g0 - m * NU, m_next, finish, lambda r0, r1: start_until(n0 + r1))
                else:
                    def step(g, carry, m=m, m_next=m_next, finish=finish, srcs=srcs):
                        def starts(r0, r1):
                            for r in range(r0, r1):
                                p, prio = piece_at(r)
                                kv_copy(srcs[r], g + (_LOOK + p // GS - srcs[r] * NU),
                                        p % GS).start(priority=prio)
                        unit(m, g - m * NU, m_next, finish, starts)
                        return carry
                    lax.fori_loop(g0, g1, step, 0)
                    pos[0] += (g1 - g0) * GS
                g0 = g1

            acc = [None] * ND

            def mac(tile, col, t):
                tr, tc = divmod(t, ND)
                prod = tile.astype(_F32) * col[tr * 8:(tr + 1) * 8, :]
                acc[tc] = prod if acc[tc] is None else acc[tc] + prod

            n0 = pos[0]
            g_sync = len(o_groups) - len(_TAIL) - 6
            n_sync = O0 + o_groups[g_sync][1] + _LANDED
            for g, (a, b) in enumerate(o_groups):
                n = n0 + (n_sync - n0) * g // g_sync if g < g_sync else 0
                start_until(min(NTOT, max(n, O0 + b + _LANDED)))
                wait_filled(wo_b.at[pl.ds(a * _PT, (b - a) * _PT)], osem.at[g])
                if g < 16:
                    for t in range(NFT * g // 16, NFT * (g + 1) // 16):
                        mac(f_b[2, t], h_s, t)
                for j in range(a, b):
                    for k in range(_PT):
                        mac(wo_b[j * _PT + k], o_s, o_list[j][1] + k)
            out_ref[0] = jnp.concatenate([jnp.sum(a, axis=0, keepdims=True) for a in acc],
                                         axis=1).astype(out_ref.dtype)

        pl.run_scoped(body, pltpu.SemaphoreType.DMA((4,)), pltpu.SemaphoreType.DMA((_SLOTS,)),
                      pltpu.SemaphoreType.DMA((len(o_groups),)))

    hbm = pl.BlockSpec(memory_space=pl.ANY)
    return pl.pallas_call(
        kernel,
        out_shape=jax.ShapeDtypeStruct((B, Sq, D), A_x.dtype),
        in_specs=[hbm] * 9,
        out_specs=pl.BlockSpec(memory_space=pltpu.VMEM),
        scratch_shapes=[
            pltpu.VMEM((_SLOTS, DH, _CW), _BF16),
            pltpu.VMEM((D, H * DH), _BF16),
            pltpu.VMEM((3, NFT, 8, 128), _BF16),
            pltpu.VMEM((NQT, 8, 128), _BF16),
            pltpu.VMEM((1, 1, D), _BF16),
            pltpu.VMEM((D,), _BF16),
            pltpu.VMEM((8, H * DH), _BF16),
            pltpu.VMEM((H, 8, DH), _BF16),
            pltpu.VMEM((NU, 8, _CW), _F32),
            pltpu.VMEM((H, 8, 128), _F32),
            pltpu.VMEM((H, 8, 128), _F32),
            pltpu.VMEM((H * DH, 128), _F32),
            pltpu.VMEM((D, 128), _F32),
            pltpu.VMEM((F, 128), _F32),
        ],
        compiler_params=pltpu.CompilerParams(vmem_limit_bytes=48 * 1024 * 1024),
    )(A_x, kT, vT, A_wq, _tiles(A_wo), _tiles(B_w1), _tiles(B_w3), _tiles(B_w2), gate_w)
```

```python
import jax
import jax.numpy as jnp
from jax import lax
import jax.experimental.pallas as pl
import jax.experimental.pallas.tpu as pltpu

_F32 = jnp.float32
_BF16 = jnp.bfloat16

_PRIO = (0, 1, 1, 1)
_AHEAD = 32
_LANDED = 64
_LOOK = 10
_SLOTS = 16
_CW = 1024
_PT = _CW // 128
_STRIDE = 256
_TAIL = (8, 4, 3)


def _tiles(a):
    R, C = a.shape
    return a.reshape(R // 8, 8, C // 128, 128).transpose(0, 2, 1, 3).reshape(-1, 8, 128)


def _even_odd(l):
    return l[0::2] + l[1::2]


def _passes(*ntiles):
    return [p for c in range(0, _STRIDE, _PT)
            for p in _even_odd([(a, t) for a, n in enumerate(ntiles) for t in range(c, n, _STRIDE)])]


@jax.jit
def pallas_gated_mix__sliding_block_cached__glu_gated_swiglu__decode_kernel(
    A_x: jax.Array,
    A_k_cache: jax.Array,
    A_v_cache: jax.Array,
    A_wq: jax.Array,
    A_wo: jax.Array,
    B_x: jax.Array,
    B_w1: jax.Array,
    B_w3: jax.Array,
    B_w2: jax.Array,
    gate_w: jax.Array,
):
    del B_x
    B, Sq, D = A_x.shape
    _, H, SK, DH = A_k_cache.shape
    F = B_w1.shape[1]
    W = min(4096, max(256, SK // 4))
    scale = DH ** -0.5
    GS = DH // 8
    NU = W // _CW * H
    ND, NF = D // 128, F // 128
    NQT, NFT = D * H * DH // 1024, D * F // 1024
    PER = len(_PRIO)
    assert B == 1 and Sq == 1 and A_wq.shape[1] == H * DH
    assert H & (H - 1) == 0 and _SLOTS & (_SLOTS - 1) == 0 and NU % _SLOTS == 0
    assert W % _CW == 0 and SK % _CW == 0 and (H * DH) % _CW == 0 and NFT % _PT == 0
    assert _AHEAD % PER == 0 and GS % PER == 0 and _PRIO[0] == 0
    assert _LOOK + pl.cdiv(_AHEAD, GS) < _SLOTS

    kT = jnp.swapaxes(A_k_cache, 2, 3).reshape(H * DH, SK)
    vT = jnp.swapaxes(A_v_cache, 2, 3).reshape(H * DH, SK)

    q_list = _passes(NQT)
    f_list = _passes(NFT, NFT, NFT)
    o_list = _passes(NQT)
    F0 = len(q_list)
    K0 = F0 + len(f_list)
    O0 = K0 + 2 * NU * GS
    NTOT = O0 + len(o_list)
    assert K0 % PER == 0
    last = len(o_list) - sum(_TAIL)
    ends = list(range(NQT // _STRIDE, last, NQT // _STRIDE)) + [last]
    for n in _TAIL:
        ends.append(ends[-1] + n)
    o_groups = list(zip([0] + ends[:-1], ends))
    o_group_of = [g for g, (a, b) in enumerate(o_groups) for _ in range(a, b)]

    def kernel(x_ref, k_ref, v_ref, wq_ref, wo_ref, w1_ref, w3_ref, w2_ref, gw_ref, out_ref,
               kv_b, wq_b, f_b, wo_b, x_b, gw_b, q_f, q_s, s_s, m_s, l_s, o_s, x_s, h_s):

        def body(wsem, kvsem, osem):
            def aligned(i, n):
                return i if isinstance(i, int) else pl.multiple_of(i, n)

            def kv_copy(m, u, r):
                r = _even_odd(list(range(GS)))[r]
                row = aligned((u & (H - 1)) * DH + r * 8, 8)
                col = aligned(SK - W + (u >> (H.bit_length() - 1)) * _CW, _CW)
                slot = u & (_SLOTS - 1)
                return pltpu.make_async_copy((k_ref, v_ref)[m].at[pl.ds(row, 8), pl.ds(col, _CW)],
                                             kv_b.at[slot, pl.ds(r * 8, 8)], kvsem.at[slot])

            def copy(i):
                if i < F0:
                    tr, tc = divmod(q_list[i][1], H * DH // 128)
                    idx = (pl.ds(tr * 8, 8), pl.ds(tc * 128, _CW))
                    return pltpu.make_async_copy(wq_ref.at[idx], wq_b.at[idx], wsem.at[0])
                if i < K0:
                    a, t = f_list[i - F0]
                    return pltpu.make_async_copy((w1_ref, w3_ref, w2_ref)[a].at[pl.ds(t, _PT)],
                                                 f_b.at[a, pl.ds(t, _PT)], wsem.at[1])
                if i < O0:
                    m, j = divmod(i - K0, NU * GS)
                    return kv_copy(m, j // GS, j % GS)
                j = i - O0
                return pltpu.make_async_copy(wo_ref.at[pl.ds(o_list[j][1], _PT)],
                                             wo_b.at[pl.ds(j * _PT, _PT)], osem.at[o_group_of[j]])

            def piece_at(i):
                return (i, 0) if _PRIO[i % PER] == 0 else (i + _AHEAD, 1)

            pos = [0]

            def start_until(n):
                while pos[0] < n:
                    p, prio = piece_at(pos[0])
                    if p < NTOT:
                        copy(p).start(priority=prio)
                    pos[0] += 1

            def wait_filled(buf, sem):
                pltpu.make_async_copy(buf, buf, sem).wait()

            def run_tasks(tasks, n_end, w0, w1):
                n0, nt = pos[0], len(tasks)
                for k, task in enumerate(tasks):
                    task()
                    start_until(n0 + (n_end - n0) * (k + 1) // nt)
                    for i in range(w0 + (w1 - w0) * k // nt, w0 + (w1 - w0) * (k + 1) // nt):
                        copy(i).wait()

            start_until(1)
            for p in range(_AHEAD):
                if _PRIO[p % PER]:
                    copy(p).start(priority=1)
            x_copy = pltpu.make_async_copy(x_ref, x_b, wsem.at[2])
            gw_copy = pltpu.make_async_copy(gw_ref, gw_b, wsem.at[3])
            x_copy.start(priority=1)
            gw_copy.start(priority=1)
            m_s[...] = jnp.full(m_s.shape, -jnp.inf, _F32)
            l_s[...] = jnp.zeros(l_s.shape, _F32)
            o_s[...] = jnp.zeros(o_s.shape, _F32)
            start_until(F0 * 5 // 8)
            x_copy.wait()
            x = x_b[0]
            xb = jnp.broadcast_to(x, (8, D))
            xf = x.astype(_F32)
            for c in range(0, D, 128):
                x_s[c:c + 128, :] = jnp.transpose(jnp.broadcast_to(xf[:, c:c + 128], (128, 128)))
            start_until(F0 * 5 // 6)
            gw_copy.wait()
            gw = gw_b[...].reshape(1, D).astype(_F32)
            gate = jax.nn.sigmoid(jnp.sum(xf * gw, axis=-1, keepdims=True))
            start_until(F0 + _LANDED)
            wait_filled(wq_b, wsem.at[0])

            def q_task(n0):
                def run():
                    q_f[:, n0:n0 + 512] = jnp.dot(xb, wq_b[:, n0:n0 + 512],
                                                  preferred_element_type=_F32).astype(_BF16)
                return run

            def q_split(h0, h1):
                def run():
                    for h in range(h0, h1):
                        q_s[h] = q_f[:, h * DH:(h + 1) * DH]
                return run

            run_tasks([q_task(n0) for n0 in range(0, H * DH, 512)]
                      + [q_split(H * i // 3, H * (i + 1) // 3) for i in range(3)],
                      K0 + _LANDED, F0, K0)

            def up_task(j):
                def run():
                    r = []
                    for a in range(2):
                        acc = [None, None]
                        for tr in range(D // 8):
                            t = f_b[a, tr * NF + j].astype(_F32) * x_s[tr * 8:(tr + 1) * 8, :]
                            acc[tr % 2] = t if acc[tr % 2] is None else acc[tr % 2] + t
                        r.append(jnp.sum(acc[0] + acc[1], axis=0, keepdims=True))
                    hh = (r[0] * jax.nn.sigmoid(r[0]) * r[1]).astype(_BF16).astype(_F32)
                    h_s[j * 128:(j + 1) * 128, :] = jnp.transpose(
                        jnp.broadcast_to(hh * (1.0 - gate), (128, 128)))
                return run

            run_tasks([up_task(j) for j in range(NF)], K0 + _LOOK * GS, K0, K0 + GS)

            def unit(m, u, m_next, finish, starts):
                h = u & (H - 1)
                buf = kv_b.at[u & (_SLOTS - 1)]

                def wait_next(r0, r1):
                    if m_next is not None:
                        for r in range(r0, r1):
                            kv_copy(m_next, (u + 1) & (NU - 1), r).wait()

                if m == 0:
                    mm = m_s[h]
                    cw = _CW // 4
                    for c in range(4):
                        s = jnp.dot(q_s[h], buf[:, c * cw:(c + 1) * cw],
                                    preferred_element_type=_F32) * scale
                        s_s[u, :, c * cw:(c + 1) * cw] = s
                        for k in range(cw // 128):
                            mm = jnp.maximum(mm, s[:, k * 128:(k + 1) * 128])
                        starts(GS * c // 4, GS * (c + 1) // 4)
                    slot = (u + 1) & (_SLOTS - 1)
                    wait_filled(kv_b.at[slot], kvsem.at[slot])
                    m_s[h] = jnp.broadcast_to(jnp.max(mm, axis=-1, keepdims=True), (8, 128))
                    return

                mx = m_s[h]
                e = [jnp.exp(s_s[u, :, k * 128:(k + 1) * 128] - mx) for k in range(_PT)]
                ll = l_s[h]
                for t in e:
                    ll = ll + t
                l_s[h] = ll
                nc = 5 if finish else 6
                for c in range(nc):
                    for r in range(GS * c // nc, GS * (c + 1) // nc):
                        rows = pl.ds(aligned(h * DH + r * 8, 8), 8)
                        vv = buf[r * 8:(r + 1) * 8, :].astype(_F32)
                        acc = [o_s[rows, :], None]
                        for k in range(_PT):
                            t = vv[:, k * 128:(k + 1) * 128] * e[k]
                            acc[k % 2] = t if acc[k % 2] is None else acc[k % 2] + t
                        o_s[rows, :] = acc[0] + acc[1]
                    starts(GS * c // 6, GS * (c + 1) // 6)
                    wait_next(GS * c // 6, GS * (c + 1) // 6)
                if finish:
                    rows = pl.ds(aligned(h * DH, 8), DH)
                    den = jnp.sum(ll, axis=-1, keepdims=True)[0:1]
                    o = jnp.sum(o_s[rows, :], axis=-1, keepdims=True) / den
                    o_s[rows, :] = jnp.broadcast_to(o.astype(_BF16).astype(_F32) * gate, (DH, 128))
                    starts(GS * 5 // 6, GS)
                    wait_next(GS * 5 // 6, GS)

            def signature(g):
                srcs = []
                for r in range(GS):
                    p, _ = piece_at(K0 + (g + _LOOK) * GS + r)
                    srcs.append((p - K0) // (NU * GS) if p < O0 else -p)
                m_next = (g + 1) // NU if g + 1 < 2 * NU else None
                return g // NU, (m_next if g >= NU else 0), g >= 2 * NU - H, tuple(srcs)

            g0 = 0
            while g0 < 2 * NU:
                sig = signature(g0)
                g1 = g0 + 1
                while g1 < 2 * NU and signature(g1) == sig:
                    g1 += 1
                m, m_next, finish, srcs = sig
                n0 = K0 + (g0 + _LOOK) * GS
                assert pos[0] == n0
                if g1 == g0 + 1:
                    unit(m, g0 - m * NU, m_next, finish, lambda r0, r1: start_until(n0 + r1))
                else:
                    def step(g, carry, m=m, m_next=m_next, finish=finish, srcs=srcs):
                        def starts(r0, r1):
                            for r in range(r0, r1):
                                p, prio = piece_at(r)
                                kv_copy(srcs[r], g + (_LOOK + p // GS - srcs[r] * NU),
                                        p % GS).start(priority=prio)
                        unit(m, g - m * NU, m_next, finish, starts)
                        return carry
                    lax.fori_loop(g0, g1, step, 0)
                    pos[0] += (g1 - g0) * GS
                g0 = g1

            acc = [None] * ND

            def mac(tile, col, t):
                tr, tc = divmod(t, ND)
                prod = tile.astype(_F32) * col[tr * 8:(tr + 1) * 8, :]
                acc[tc] = prod if acc[tc] is None else acc[tc] + prod

            n0 = pos[0]
            g_sync = len(o_groups) - len(_TAIL) - 6
            n_sync = O0 + o_groups[g_sync][1] + _LANDED
            for g, (a, b) in enumerate(o_groups):
                n = n0 + (n_sync - n0) * g // g_sync if g < g_sync else 0
                start_until(min(NTOT, max(n, O0 + b + _LANDED)))
                wait_filled(wo_b.at[pl.ds(a * _PT, (b - a) * _PT)], osem.at[g])
                if g < 16:
                    for t in range(NFT * g // 16, NFT * (g + 1) // 16):
                        mac(f_b[2, t], h_s, t)
                for j in range(a, b):
                    for k in range(_PT):
                        mac(wo_b[j * _PT + k], o_s, o_list[j][1] + k)
            out_ref[0] = jnp.concatenate([jnp.sum(a, axis=0, keepdims=True) for a in acc],
                                         axis=1).astype(out_ref.dtype)

        pl.run_scoped(body, pltpu.SemaphoreType.DMA((4,)), pltpu.SemaphoreType.DMA((_SLOTS,)),
                      pltpu.SemaphoreType.DMA((len(o_groups),)))

    hbm = pl.BlockSpec(memory_space=pl.ANY)
    return pl.pallas_call(
        kernel,
        out_shape=jax.ShapeDtypeStruct((B, Sq, D), A_x.dtype),
        in_specs=[hbm] * 9,
        out_specs=pl.BlockSpec(memory_space=pltpu.VMEM),
        scratch_shapes=[
            pltpu.VMEM((_SLOTS, DH, _CW), _BF16),
            pltpu.VMEM((D, H * DH), _BF16),
            pltpu.VMEM((3, NFT, 8, 128), _BF16),
            pltpu.VMEM((NQT, 8, 128), _BF16),
            pltpu.VMEM((1, 1, D), _BF16),
            pltpu.VMEM((D,), _BF16),
            pltpu.VMEM((8, H * DH), _BF16),
            pltpu.VMEM((H, 8, DH), _BF16),
            pltpu.VMEM((NU, 8, _CW), _F32),
            pltpu.VMEM((H, 8, 128), _F32),
            pltpu.VMEM((H, 8, 128), _F32),
            pltpu.VMEM((H * DH, 128), _F32),
            pltpu.VMEM((D, 128), _F32),
            pltpu.VMEM((F, 128), _F32),
        ],
        compiler_params=pltpu.CompilerParams(vmem_limit_bytes=48 * 1024 * 1024),
    )(A_x, kT, vT, A_wq, _tiles(A_wo), _tiles(B_w1), _tiles(B_w3), _tiles(B_w2), gate_w)
```

```python
import jax
import jax.numpy as jnp
from jax import lax
import jax.experimental.pallas as pl
import jax.experimental.pallas.tpu as pltpu

_F32 = jnp.float32
_BF16 = jnp.bfloat16

_PRIO = (0, 1, 1, 1)
_KV_ROW = (0, 2, 1 - 16, 3 - 16)
_AHEAD = 32
_LANDED = 64
_LOOK = 10
_SLOTS = 16
_CW = 1024
_PT = _CW // 128
_STRIDE = 256
_GROUP = 15
_TAIL = (4,) * 14 + (2, 2)
_CONTIG = 32
_FLIGHT = 30


def _tiles(a):
    R, C = a.shape
    return a.reshape(R // 8, 8, C // 128, 128).transpose(0, 2, 1, 3).reshape(-1, 8, 128)


def _even_odd(l):
    return l[0::2] + l[1::2]


def _passes(*ntiles):
    return [p for c in range(0, _STRIDE, _PT)
            for p in _even_odd([(a, t) for a, n in enumerate(ntiles) for t in range(c, n, _STRIDE)])]


@jax.jit
def pallas_gated_mix__sliding_block_cached__glu_gated_swiglu__decode_kernel(
    A_x: jax.Array,
    A_k_cache: jax.Array,
    A_v_cache: jax.Array,
    A_wq: jax.Array,
    A_wo: jax.Array,
    B_x: jax.Array,
    B_w1: jax.Array,
    B_w3: jax.Array,
    B_w2: jax.Array,
    gate_w: jax.Array,
):
    del B_x
    B, Sq, D = A_x.shape
    _, H, SK, DH = A_k_cache.shape
    F = B_w1.shape[1]
    W = min(4096, max(256, SK // 4))
    scale = DH ** -0.5
    GS = DH // 8
    NU = W // _CW * H
    ND, NF = D // 128, F // 128
    NQT, NFT = D * H * DH // 1024, D * F // 1024
    PER = len(_PRIO)
    assert B == 1 and Sq == 1 and A_wq.shape[1] == H * DH
    assert H & (H - 1) == 0 and _SLOTS & (_SLOTS - 1) == 0 and NU % _SLOTS == 0
    assert W % _CW == 0 and SK % _CW == 0 and (H * DH) % _CW == 0 and NFT % _PT == 0
    assert _AHEAD % PER == 0 and GS % PER == 0 and _PRIO[0] == 0
    assert sorted(r % PER for r in _KV_ROW) == list(range(PER)) and max(_KV_ROW) < PER
    assert _LOOK + pl.cdiv(_AHEAD, GS) < _SLOTS

    kT = jnp.swapaxes(A_k_cache, 2, 3).reshape(H * DH, SK)
    vT = jnp.swapaxes(A_v_cache, 2, 3).reshape(H * DH, SK)

    q_list = _passes(NQT)
    f_list = _passes(NFT, NFT, NFT)
    o_list = _passes(NQT - _CONTIG * _PT) + [(0, t) for t in range(NQT - _CONTIG * _PT, NQT, _PT)]
    F0 = len(q_list)
    K0 = F0 + len(f_list)
    O0 = K0 + 2 * NU * GS - min(_KV_ROW) // PER * PER
    NTOT = O0 + len(o_list)
    assert K0 % PER == 0
    ends = list(range(len(o_list) - sum(_TAIL), 0, -_GROUP))[::-1]
    for n in _TAIL:
        ends.append(ends[-1] + n)
    o_groups = list(zip([0] + ends[:-1], ends))
    o_group_of = [g for g, (a, b) in enumerate(o_groups) for _ in range(a, b)]

    def kernel(x_ref, k_ref, v_ref, wq_ref, wo_ref, w1_ref, w3_ref, w2_ref, gw_ref, out_ref,
               kv_b, wq_b, f_b, wo_b, x_b, gw_b, q_f, q_s, s_s, m_s, l_s, o_s, x_s, h_s):

        def body(wsem, kvsem, osem):
            def aligned(i, n):
                return i if isinstance(i, int) else pl.multiple_of(i, n)

            def kv_copy(m, u, r):
                row = aligned((u & (H - 1)) * DH + r * 8, 8)
                col = aligned(SK - W + (u >> (H.bit_length() - 1)) * _CW, _CW)
                slot = u & (_SLOTS - 1)
                return pltpu.make_async_copy((k_ref, v_ref)[m].at[pl.ds(row, 8), pl.ds(col, _CW)],
                                             kv_b.at[slot, pl.ds(r * 8, 8)], kvsem.at[slot])

            def kv_row(j):
                return j - j % PER + _KV_ROW[j % PER]

            def copy(i):
                if i < F0:
                    tr, tc = divmod(q_list[i][1], H * DH // 128)
                    idx = (pl.ds(tr * 8, 8), pl.ds(tc * 128, _CW))
                    return pltpu.make_async_copy(wq_ref.at[idx], wq_b.at[idx], wsem.at[0])
                if i < K0:
                    a, t = f_list[i - F0]
                    return pltpu.make_async_copy((w1_ref, w3_ref, w2_ref)[a].at[pl.ds(t, _PT)],
                                                 f_b.at[a, pl.ds(t, _PT)], wsem.at[1])
                if i < O0:
                    m, j = divmod(kv_row(i - K0), NU * GS)
                    return kv_copy(m, j // GS, j % GS) if m in (0, 1) else None
                j = i - O0
                return pltpu.make_async_copy(wo_ref.at[pl.ds(o_list[j][1], _PT)],
                                             wo_b.at[pl.ds(j * _PT, _PT)], osem.at[o_group_of[j]])

            def piece_at(i):
                return (i, 0) if _PRIO[i % PER] == 0 else (i + _AHEAD, 1)

            pos = [0]

            def start_until(n):
                while pos[0] < n:
                    p, prio = piece_at(pos[0])
                    cp = copy(p) if p < NTOT else None
                    if cp is not None:
                        cp.start(priority=prio)
                    pos[0] += 1

            def wait_filled(buf, sem):
                pltpu.make_async_copy(buf, buf, sem).wait()

            def run_tasks(tasks, n_end, group):
                n0, nt, nw = pos[0], len(tasks), len(group)
                for k, task in enumerate(tasks):
                    task()
                    start_until(n0 + (n_end - n0) * (k + 1) // nt)
                    for cp in group[nw * k // nt:nw * (k + 1) // nt]:
                        cp.wait()

            start_until(1)
            for p in range(_AHEAD):
                if _PRIO[p % PER]:
                    copy(p).start(priority=1)
            x_copy = pltpu.make_async_copy(x_ref, x_b, wsem.at[2])
            gw_copy = pltpu.make_async_copy(gw_ref, gw_b, wsem.at[3])
            x_copy.start(priority=1)
            gw_copy.start(priority=1)
            m_s[...] = jnp.full(m_s.shape, -jnp.inf, _F32)
            l_s[...] = jnp.zeros(l_s.shape, _F32)
            o_s[...] = jnp.zeros(o_s.shape, _F32)
            start_until(F0 * 5 // 8)
            x_copy.wait()
            x = x_b[0]
            xb = jnp.broadcast_to(x, (8, D))
            xf = x.astype(_F32)
            for c in range(0, D, 128):
                x_s[c:c + 128, :] = jnp.transpose(jnp.broadcast_to(xf[:, c:c + 128], (128, 128)))
            start_until(F0 * 5 // 6)
            gw_copy.wait()
            gw = gw_b[...].reshape(1, D).astype(_F32)
            gate = jax.nn.sigmoid(jnp.sum(xf * gw, axis=-1, keepdims=True))
            start_until(F0 + _LANDED)
            wait_filled(wq_b, wsem.at[0])

            def q_task(n0):
                def run():
                    q_f[:, n0:n0 + 512] = jnp.dot(xb, wq_b[:, n0:n0 + 512],
                                                  preferred_element_type=_F32).astype(_BF16)
                return run

            def q_split(h0, h1):
                def run():
                    for h in range(h0, h1):
                        q_s[h] = q_f[:, h * DH:(h + 1) * DH]
                return run

            run_tasks([q_task(n0) for n0 in range(0, H * DH, 512)]
                      + [q_split(H * i // 3, H * (i + 1) // 3) for i in range(3)],
                      K0 + _LANDED, [copy(i) for i in range(F0, K0)])

            def up_task(j):
                def run():
                    r = []
                    for a in range(2):
                        acc = [None, None]
                        for tr in range(D // 8):
                            t = f_b[a, tr * NF + j].astype(_F32) * x_s[tr * 8:(tr + 1) * 8, :]
                            acc[tr % 2] = t if acc[tr % 2] is None else acc[tr % 2] + t
                        r.append(jnp.sum(acc[0] + acc[1], axis=0, keepdims=True))
                    hh = (r[0] * jax.nn.sigmoid(r[0]) * r[1]).astype(_BF16).astype(_F32)
                    h_s[j * 128:(j + 1) * 128, :] = jnp.transpose(
                        jnp.broadcast_to(hh * (1.0 - gate), (128, 128)))
                return run

            run_tasks([up_task(j) for j in range(NF)], K0 + _LOOK * GS,
                      [kv_copy(0, 0, r) for r in range(GS)])

            def unit(m, u, m_next, finish, starts):
                h = u & (H - 1)
                buf = kv_b.at[u & (_SLOTS - 1)]

                def wait_next(r0, r1):
                    if m_next is not None:
                        for r in range(r0, r1):
                            kv_copy(m_next, (u + 1) & (NU - 1), r).wait()

                if m == 0:
                    mm = m_s[h]
                    cw = _CW // 4
                    for c in range(4):
                        s = jnp.dot(q_s[h], buf[:, c * cw:(c + 1) * cw],
                                    preferred_element_type=_F32) * scale
                        s_s[u, :, c * cw:(c + 1) * cw] = s
                        for k in range(cw // 128):
                            mm = jnp.maximum(mm, s[:, k * 128:(k + 1) * 128])
                        starts(GS * c // 4, GS * (c + 1) // 4)
                    slot = (u + 1) & (_SLOTS - 1)
                    wait_filled(kv_b.at[slot], kvsem.at[slot])
                    m_s[h] = jnp.broadcast_to(jnp.max(mm, axis=-1, keepdims=True), (8, 128))
                    return

                mx = m_s[h]
                e = [jnp.exp(s_s[u, :, k * 128:(k + 1) * 128] - mx) for k in range(_PT)]
                ll = l_s[h]
                for t in e:
                    ll = ll + t
                l_s[h] = ll
                nc = 5 if finish else 6
                for c in range(nc):
                    for r in range(GS * c // nc, GS * (c + 1) // nc):
                        rows = pl.ds(aligned(h * DH + r * 8, 8), 8)
                        vv = buf[r * 8:(r + 1) * 8, :].astype(_F32)
                        acc = [o_s[rows, :], None]
                        for k in range(_PT):
                            t = vv[:, k * 128:(k + 1) * 128] * e[k]
                            acc[k % 2] = t if acc[k % 2] is None else acc[k % 2] + t
                        o_s[rows, :] = acc[0] + acc[1]
                    starts(GS * c // 6, GS * (c + 1) // 6)
                    wait_next(GS * c // 6, GS * (c + 1) // 6)
                if finish:
                    rows = pl.ds(aligned(h * DH, 8), DH)
                    den = jnp.sum(ll, axis=-1, keepdims=True)[0:1]
                    o = jnp.sum(o_s[rows, :], axis=-1, keepdims=True) / den
                    o_s[rows, :] = jnp.broadcast_to(o.astype(_BF16).astype(_F32) * gate, (DH, 128))
                    starts(GS * 5 // 6, GS)
                    wait_next(GS * 5 // 6, GS)

            def signature(g):
                srcs = []
                for r in range(GS):
                    p, _ = piece_at(K0 + (g + _LOOK) * GS + r)
                    m = kv_row(p - K0) // (NU * GS)
                    srcs.append(m if m in (0, 1) else -p)
                m_next = (g + 1) // NU if g + 1 < 2 * NU else None
                return g // NU, (m_next if g >= NU else 0), g >= 2 * NU - H, tuple(srcs)

            g0 = 0
            while g0 < 2 * NU:
                sig = signature(g0)
                g1 = g0 + 1
                while g1 < 2 * NU and signature(g1) == sig:
                    g1 += 1
                m, m_next, finish, srcs = sig
                n0 = K0 + (g0 + _LOOK) * GS
                assert pos[0] == n0
                if g1 == g0 + 1:
                    unit(m, g0 - m * NU, m_next, finish, lambda r0, r1: start_until(n0 + r1))
                else:
                    def step(g, carry, m=m, m_next=m_next, finish=finish, srcs=srcs):
                        def starts(r0, r1):
                            for r in range(r0, r1):
                                p, prio = piece_at(r)
                                du, row = divmod(kv_row(p), GS)
                                kv_copy(srcs[r], g + (_LOOK + du - srcs[r] * NU),
                                        row).start(priority=prio)
                        unit(m, g - m * NU, m_next, finish, starts)
                        return carry
                    lax.fori_loop(g0, g1, step, 0)
                    pos[0] += (g1 - g0) * GS
                g0 = g1

            acc = [None] * ND

            def mac(tile, col, t):
                tr, tc = divmod(t, ND)
                prod = tile.astype(_F32) * col[tr * 8:(tr + 1) * 8, :]
                acc[tc] = prod if acc[tc] is None else acc[tc] + prod

            n0 = pos[0]
            g_sync = len(o_groups) - len(_TAIL) - 6
            n_sync = O0 + o_groups[g_sync][1] + _LANDED
            for g, (a, b) in enumerate(o_groups):
                n = n0 + (n_sync - n0) * g // g_sync if g < g_sync else 0
                n = max(n, O0 + b + _LANDED)
                if n > NTOT - _AHEAD:
                    n = max(NTOT - _AHEAD, O0 + b + _FLIGHT)
                start_until(min(NTOT, n))
                wait_filled(wo_b.at[pl.ds(a * _PT, (b - a) * _PT)], osem.at[g])
                if g < 16:
                    for t in range(NFT * g // 16, NFT * (g + 1) // 16):
                        mac(f_b[2, t], h_s, t)
                for j in range(a, b):
                    for k in range(_PT):
                        mac(wo_b[j * _PT + k], o_s, o_list[j][1] + k)
            out_ref[0] = jnp.concatenate([jnp.sum(a, axis=0, keepdims=True) for a in acc],
                                         axis=1).astype(out_ref.dtype)

        pl.run_scoped(body, pltpu.SemaphoreType.DMA((4,)), pltpu.SemaphoreType.DMA((_SLOTS,)),
                      pltpu.SemaphoreType.DMA((len(o_groups),)))

    hbm = pl.BlockSpec(memory_space=pl.ANY)
    return pl.pallas_call(
        kernel,
        out_shape=jax.ShapeDtypeStruct((B, Sq, D), A_x.dtype),
        in_specs=[hbm] * 9,
        out_specs=pl.BlockSpec(memory_space=pltpu.VMEM),
        scratch_shapes=[
            pltpu.VMEM((_SLOTS, DH, _CW), _BF16),
            pltpu.VMEM((D, H * DH), _BF16),
            pltpu.VMEM((3, NFT, 8, 128), _BF16),
            pltpu.VMEM((NQT, 8, 128), _BF16),
            pltpu.VMEM((1, 1, D), _BF16),
            pltpu.VMEM((D,), _BF16),
            pltpu.VMEM((8, H * DH), _BF16),
            pltpu.VMEM((H, 8, DH), _BF16),
            pltpu.VMEM((NU, 8, _CW), _F32),
            pltpu.VMEM((H, 8, 128), _F32),
            pltpu.VMEM((H, 8, 128), _F32),
            pltpu.VMEM((H * DH, 128), _F32),
            pltpu.VMEM((D, 128), _F32),
            pltpu.VMEM((F, 128), _F32),
        ],
        compiler_params=pltpu.CompilerParams(vmem_limit_bytes=48 * 1024 * 1024),
    )(A_x, kT, vT, A_wq, _tiles(A_wo), _tiles(B_w1), _tiles(B_w3), _tiles(B_w2), gate_w)
```

```python
import jax
import jax.numpy as jnp
from jax import lax
import jax.experimental.pallas as pl
import jax.experimental.pallas.tpu as pltpu

_F32 = jnp.float32
_BF16 = jnp.bfloat16

_PRIO = (0, 1, 1, 1)
_KV_ROW = (-4, -15, 2, -13)
_AHEAD = 32
_LANDED = 64
_LOOK = 10
_SLOTS = 16
_CW = 1024
_PT = _CW // 128
_STRIDE = 256
_GROUP = 15
_TAIL = (4,) * 14 + (2, 2)
_CONTIG = 32
_FLIGHT = 30


def _tiles(a):
    R, C = a.shape
    return a.reshape(R // 8, 8, C // 128, 128).transpose(0, 2, 1, 3).reshape(-1, 8, 128)


def _even_odd(l):
    return l[0::2] + l[1::2]


def _passes(*ntiles):
    return [p for c in range(0, _STRIDE, _PT)
            for p in _even_odd([(a, t) for a, n in enumerate(ntiles) for t in range(c, n, _STRIDE)])]


@jax.jit
def pallas_gated_mix__sliding_block_cached__glu_gated_swiglu__decode_kernel(
    A_x: jax.Array,
    A_k_cache: jax.Array,
    A_v_cache: jax.Array,
    A_wq: jax.Array,
    A_wo: jax.Array,
    B_x: jax.Array,
    B_w1: jax.Array,
    B_w3: jax.Array,
    B_w2: jax.Array,
    gate_w: jax.Array,
):
    del B_x
    B, Sq, D = A_x.shape
    _, H, SK, DH = A_k_cache.shape
    F = B_w1.shape[1]
    W = min(4096, max(256, SK // 4))
    scale = DH ** -0.5
    GS = DH // 8
    NU = W // _CW * H
    ND, NF = D // 128, F // 128
    NQT, NFT = D * H * DH // 1024, D * F // 1024
    PER = len(_PRIO)
    assert B == 1 and Sq == 1 and A_wq.shape[1] == H * DH
    assert H & (H - 1) == 0 and _SLOTS & (_SLOTS - 1) == 0 and NU % _SLOTS == 0
    assert W % _CW == 0 and SK % _CW == 0 and (H * DH) % _CW == 0 and NFT % _PT == 0
    assert _AHEAD % PER == 0 and GS % PER == 0 and _PRIO[0] == 0
    assert sorted(r % PER for r in _KV_ROW) == list(range(PER)) and max(_KV_ROW) < PER
    assert _LOOK + pl.cdiv(_AHEAD, GS) < _SLOTS

    kT = jnp.swapaxes(A_k_cache, 2, 3).reshape(H * DH, SK)
    vT = jnp.swapaxes(A_v_cache, 2, 3).reshape(H * DH, SK)

    q_list = _passes(NQT)
    f_list = _passes(NFT, NFT, NFT)
    o_list = _passes(NQT - _CONTIG * _PT) + [(0, t) for t in range(NQT - _CONTIG * _PT, NQT, _PT)]
    F0 = len(q_list)
    K0 = F0 + len(f_list)
    O0 = K0 + 2 * NU * GS - min(_KV_ROW) // PER * PER
    NTOT = O0 + len(o_list)
    assert K0 % PER == 0
    ends = list(range(len(o_list) - sum(_TAIL), 0, -_GROUP))[::-1]
    for n in _TAIL:
        ends.append(ends[-1] + n)
    o_groups = list(zip([0] + ends[:-1], ends))
    o_group_of = [g for g, (a, b) in enumerate(o_groups) for _ in range(a, b)]

    def kernel(x_ref, k_ref, v_ref, wq_ref, wo_ref, w1_ref, w3_ref, w2_ref, gw_ref, out_ref,
               kv_b, wq_b, f_b, wo_b, x_b, gw_b, q_f, q_s, s_s, m_s, l_s, o_s, x_s, h_s):

        def body(wsem, kvsem, osem):
            def aligned(i, n):
                return i if isinstance(i, int) else pl.multiple_of(i, n)

            def kv_copy(m, u, r):
                row = aligned((u & (H - 1)) * DH + r * 8, 8)
                col = aligned(SK - W + (u >> (H.bit_length() - 1)) * _CW, _CW)
                slot = u & (_SLOTS - 1)
                return pltpu.make_async_copy((k_ref, v_ref)[m].at[pl.ds(row, 8), pl.ds(col, _CW)],
                                             kv_b.at[slot, pl.ds(r * 8, 8)], kvsem.at[slot])

            def kv_row(j):
                return j - j % PER + _KV_ROW[j % PER]

            def copy(i):
                if i < F0:
                    tr, tc = divmod(q_list[i][1], H * DH // 128)
                    idx = (pl.ds(tr * 8, 8), pl.ds(tc * 128, _CW))
                    return pltpu.make_async_copy(wq_ref.at[idx], wq_b.at[idx], wsem.at[0])
                if i < K0:
                    a, t = f_list[i - F0]
                    return pltpu.make_async_copy((w1_ref, w3_ref, w2_ref)[a].at[pl.ds(t, _PT)],
                                                 f_b.at[a, pl.ds(t, _PT)], wsem.at[1])
                if i < O0:
                    m, j = divmod(kv_row(i - K0), NU * GS)
                    return kv_copy(m, j // GS, j % GS) if m in (0, 1) else None
                idx = pl.ds(o_list[i - O0][1], _PT)
                return pltpu.make_async_copy(wo_ref.at[idx], wo_b.at[idx],
                                             osem.at[o_group_of[i - O0]])

            def piece_at(i):
                return (i, 0) if _PRIO[i % PER] == 0 else (i + _AHEAD, 1)

            pos = [0]

            def start_until(n):
                while pos[0] < n:
                    p, prio = piece_at(pos[0])
                    cp = copy(p) if p < NTOT else None
                    if cp is not None:
                        cp.start(priority=prio)
                    pos[0] += 1

            def wait_filled(buf, sem):
                pltpu.make_async_copy(buf, buf, sem).wait()

            def run_tasks(tasks, n_end, group):
                n0, nt, nw = pos[0], len(tasks), len(group)
                for k, task in enumerate(tasks):
                    task()
                    start_until(n0 + (n_end - n0) * (k + 1) // nt)
                    for cp in group[nw * k // nt:nw * (k + 1) // nt]:
                        cp.wait()

            start_until(1)
            for p in range(_AHEAD):
                if _PRIO[p % PER]:
                    copy(p).start(priority=1)
            x_copy = pltpu.make_async_copy(x_ref, x_b, wsem.at[2])
            gw_copy = pltpu.make_async_copy(gw_ref, gw_b, wsem.at[3])
            x_copy.start(priority=1)
            gw_copy.start(priority=1)
            m_s[...] = jnp.full(m_s.shape, -jnp.inf, _F32)
            l_s[...] = jnp.zeros(l_s.shape, _F32)
            o_s[...] = jnp.zeros(o_s.shape, _F32)
            start_until(F0 * 5 // 8)
            x_copy.wait()
            x = x_b[0]
            xb = jnp.broadcast_to(x, (8, D))
            xf = x.astype(_F32)
            for c in range(0, D, 128):
                x_s[c:c + 128, :] = jnp.transpose(jnp.broadcast_to(xf[:, c:c + 128], (128, 128)))
            start_until(F0 * 5 // 6)
            gw_copy.wait()
            gw = gw_b[...].reshape(1, D).astype(_F32)
            gate = jax.nn.sigmoid(jnp.sum(xf * gw, axis=-1, keepdims=True))
            start_until(F0 + _LANDED)
            wait_filled(wq_b, wsem.at[0])

            def q_task(n0):
                def run():
                    q_f[:, n0:n0 + 512] = jnp.dot(xb, wq_b[:, n0:n0 + 512],
                                                  preferred_element_type=_F32).astype(_BF16)
                return run

            def q_split(h0, h1):
                def run():
                    for h in range(h0, h1):
                        q_s[h] = q_f[:, h * DH:(h + 1) * DH]
                return run

            run_tasks([q_task(n0) for n0 in range(0, H * DH, 512)]
                      + [q_split(H * i // 3, H * (i + 1) // 3) for i in range(3)],
                      K0 + _LANDED, [copy(i) for i in range(F0, K0)])

            def project(w, lead, col, r0, r1, n):
                t = w[(*lead, pl.ds(r0 * n, (r1 - r0) * n))].astype(_F32)
                c = col[r0 * 8:r1 * 8, :].reshape(r1 - r0, 1, 8, 128)
                return jnp.sum(t.reshape(r1 - r0, n, 8, 128) * c, axis=0)

            up = [0.0, 0.0]

            def up_task(r0, r1):
                def run():
                    for a in range(2):
                        up[a] = up[a] + project(f_b, (a,), x_s, r0, r1, NF)
                return run

            def act_task(j0, j1):
                def run():
                    for j in range(j0, j1):
                        g_, u_ = (jnp.sum(up[a][j], axis=0, keepdims=True) for a in range(2))
                        hh = (g_ * jax.nn.sigmoid(g_) * u_).astype(_BF16).astype(_F32)
                        h_s[j * 128:(j + 1) * 128, :] = jnp.transpose(
                            jnp.broadcast_to(hh * (1.0 - gate), (128, 128)))
                return run

            run_tasks([up_task(D // 8 * i // 8, D // 8 * (i + 1) // 8) for i in range(8)]
                      + [act_task(NF * i // 4, NF * (i + 1) // 4) for i in range(4)],
                      K0 + _LOOK * GS, [kv_copy(0, 0, r) for r in range(GS)])

            def unit(m, u, m_next, finish, starts):
                h = u & (H - 1)
                buf = kv_b.at[u & (_SLOTS - 1)]

                def wait_next(r0, r1):
                    if m_next is not None:
                        for r in range(r0, r1):
                            kv_copy(m_next, (u + 1) & (NU - 1), r).wait()

                if m == 0:
                    mm = m_s[h]
                    cw = _CW // 4
                    for c in range(4):
                        s = jnp.dot(q_s[h], buf[:, c * cw:(c + 1) * cw],
                                    preferred_element_type=_F32) * scale
                        s_s[u, :, c * cw:(c + 1) * cw] = s
                        for k in range(cw // 128):
                            mm = jnp.maximum(mm, s[:, k * 128:(k + 1) * 128])
                        starts(GS * c // 4, GS * (c + 1) // 4)
                    slot = (u + 1) & (_SLOTS - 1)
                    wait_filled(kv_b.at[slot], kvsem.at[slot])
                    m_s[h] = jnp.broadcast_to(jnp.max(mm, axis=-1, keepdims=True), (8, 128))
                    return

                def fold(t, acc):
                    for k in range(_PT):
                        acc = acc + t[:, k * 128:(k + 1) * 128]
                    return acc

                e = jnp.exp(s_s[u] - jnp.concatenate([m_s[h]] * _PT, axis=1))
                ll = fold(e, l_s[h])
                l_s[h] = ll
                nc = 4 if finish else 6
                nr = DH // nc
                for c in range(nc):
                    rows = pl.ds(aligned(h * DH + c * nr, 8), nr)
                    vv = buf[c * nr:(c + 1) * nr, :].astype(_F32)
                    o_s[rows, :] = fold(vv * jnp.concatenate([e] * (nr // 8), axis=0), o_s[rows, :])
                    starts(GS * c // 6, GS * (c + 1) // 6)
                    wait_next(GS * c // 6, GS * (c + 1) // 6)
                if finish:
                    rows = pl.ds(aligned(h * DH, 8), DH)
                    den = jnp.sum(ll, axis=-1, keepdims=True)[0:1]
                    o = jnp.sum(o_s[rows, :], axis=-1, keepdims=True) / den
                    o_s[rows, :] = jnp.broadcast_to(o.astype(_BF16).astype(_F32) * gate, (DH, 128))
                    starts(GS * nc // 6, GS)
                    wait_next(GS * nc // 6, GS)

            def signature(g):
                srcs = []
                for r in range(GS):
                    p, _ = piece_at(K0 + (g + _LOOK) * GS + r)
                    m = kv_row(p - K0) // (NU * GS)
                    srcs.append(m if m in (0, 1) else -p)
                m_next = (g + 1) // NU if g + 1 < 2 * NU else None
                return g // NU, (m_next if g >= NU else 0), g >= 2 * NU - H, tuple(srcs)

            g0 = 0
            while g0 < 2 * NU:
                sig = signature(g0)
                g1 = g0 + 1
                while g1 < 2 * NU and signature(g1) == sig:
                    g1 += 1
                m, m_next, finish, srcs = sig
                n0 = K0 + (g0 + _LOOK) * GS
                assert pos[0] == n0
                if g1 == g0 + 1:
                    unit(m, g0 - m * NU, m_next, finish, lambda r0, r1: start_until(n0 + r1))
                else:
                    def step(g, carry, m=m, m_next=m_next, finish=finish, srcs=srcs):
                        def starts(r0, r1):
                            for r in range(r0, r1):
                                p, prio = piece_at(r)
                                du, row = divmod(kv_row(p), GS)
                                kv_copy(srcs[r], g + (_LOOK + du - srcs[r] * NU),
                                        row).start(priority=prio)
                        unit(m, g - m * NU, m_next, finish, starts)
                        return carry
                    lax.fori_loop(g0, g1, step, 0)
                    pos[0] += (g1 - g0) * GS
                g0 = g1

            acc = 0.0
            missing = [ND] * (NQT // ND)
            n0 = pos[0]
            g_sync = len(o_groups) - len(_TAIL) - 6
            n_sync = O0 + o_groups[g_sync][1] + _LANDED
            for g, (a, b) in enumerate(o_groups):
                n = n0 + (n_sync - n0) * g // g_sync if g < g_sync else 0
                n = max(n, O0 + b + _LANDED)
                if n > NTOT - _AHEAD:
                    n = max(NTOT - _AHEAD, O0 + b + _FLIGHT)
                start_until(min(NTOT, n))
                ready = []
                for j in range(a, b):
                    copy(O0 + j).wait()
                    for t in range(o_list[j][1], o_list[j][1] + _PT):
                        missing[t // ND] -= 1
                        if missing[t // ND] == 0:
                            ready.append(t // ND)
                if g < g_sync:
                    acc = acc + project(f_b, (2,), h_s, F // 8 * g // g_sync,
                                        F // 8 * (g + 1) // g_sync, ND)
                ready.sort()
                firsts = [r for r in ready if r - 1 not in ready]
                lasts = [r for r in ready if r + 1 not in ready]
                for r0, r1 in zip(firsts, lasts):
                    acc = acc + project(wo_b, (), o_s, r0, r1 + 1, ND)
            assert not any(missing) and pos[0] == NTOT
            out_ref[0] = jnp.concatenate(
                [jnp.sum(acc[j], axis=0, keepdims=True) for j in range(ND)],
                axis=1).astype(out_ref.dtype)

        pl.run_scoped(body, pltpu.SemaphoreType.DMA((4,)), pltpu.SemaphoreType.DMA((_SLOTS,)),
                      pltpu.SemaphoreType.DMA((len(o_groups),)))

    hbm = pl.BlockSpec(memory_space=pl.ANY)
    return pl.pallas_call(
        kernel,
        out_shape=jax.ShapeDtypeStruct((B, Sq, D), A_x.dtype),
        in_specs=[hbm] * 9,
        out_specs=pl.BlockSpec(memory_space=pltpu.VMEM),
        scratch_shapes=[
            pltpu.VMEM((_SLOTS, DH, _CW), _BF16),
            pltpu.VMEM((D, H * DH), _BF16),
            pltpu.VMEM((3, NFT, 8, 128), _BF16),
            pltpu.VMEM((NQT, 8, 128), _BF16),
            pltpu.VMEM((1, 1, D), _BF16),
            pltpu.VMEM((D,), _BF16),
            pltpu.VMEM((8, H * DH), _BF16),
            pltpu.VMEM((H, 8, DH), _BF16),
            pltpu.VMEM((NU, 8, _CW), _F32),
            pltpu.VMEM((H, 8, 128), _F32),
            pltpu.VMEM((H, 8, 128), _F32),
            pltpu.VMEM((H * DH, 128), _F32),
            pltpu.VMEM((D, 128), _F32),
            pltpu.VMEM((F, 128), _F32),
        ],
        compiler_params=pltpu.CompilerParams(vmem_limit_bytes=48 * 1024 * 1024),
    )(A_x, kT, vT, A_wq, _tiles(A_wo), _tiles(B_w1), _tiles(B_w3), _tiles(B_w2), gate_w)
```
